```python
import os as _os
_os.environ.setdefault('JAX_PLATFORMS', 'cpu')
import jax
import jax.numpy as jnp

def _softmax(x, axis=-1):
    return jax.nn.softmax(x, axis=axis)

def _gelu(x):
    return jax.nn.gelu(x, approximate=True)

def _silu(x):
    return jax.nn.silu(x)

def _sigmoid(x):
    return jax.nn.sigmoid(x)

def _layernorm(x, axis=-1, eps=1e-05):
    m = jnp.mean(x, axis=axis, keepdims=True)
    v = jnp.var(x, axis=axis, keepdims=True)
    return (x - m) / jnp.sqrt(v + eps)

def _scatter_add(tgt, idx, src, axis=0):
    return tgt.at[idx].add(src)

def _segment_sum(src, seg, n):
    return jax.ops.segment_sum(src, seg, n)

class _Rng:

    def __init__(self, key):
        self._k = key

    def _next(self):
        self._k, sub = jax.random.split(self._k)
        return sub

    def normal(self, shape):
        return jax.random.normal(self._next(), shape, dtype=jnp.bfloat16)

    def randint(self, lo, hi, shape):
        return jax.random.randint(self._next(), shape, lo, hi, dtype=jnp.int32)

    def uniform(self, shape, lo=0.0, hi=1.0):
        return jax.random.uniform(self._next(), shape, jnp.bfloat16, lo, hi)

    def permutation(self, n):
        return jax.random.permutation(self._next(), n)
kernel_name = 'gated_mix__ssm_conv_h3__memory_aug_recurrent_mem_tr__prompt'

def setup_inputs():
    _rng = _Rng(jax.random.key(int.from_bytes(__import__("os").urandom(4), "little")))
    _w = lambda a: (lambda t: t.astype(jnp.bfloat16) if jnp.issubdtype(t.dtype, jnp.floating) else t)(jnp.asarray(a))

    def _A_setup():
        B, S, D = (1, 2048, 1024)
        ks = 4
        return {'q': _w((lambda *s: _rng.normal(s) * 0.05)(B, S, D)), 'k': _w((lambda *s: _rng.normal(s) * 0.4)(B, S, D)), 'v': _w((lambda *s: _rng.normal(s) * 0.4)(B, S, D)), 'shift_k': _w((lambda *s: _rng.normal(s) * 0.4)(D, ks) * 0.5), 'ssm_k': _w((lambda *s: _rng.normal(s) * 0.4)(D, S) * (1.0 / S ** 0.5)), 'ssm_D': _w((lambda *s: _rng.normal(s) * 0.4)(D))}
    _A_in = _A_setup()

    def _B_setup():
        B, S, Dm = (1, 2048, 1024)
        H, Dh = (32, 128)
        M, seg = (8, 32)
        seg = min(seg, S)
        S = S // seg * seg
        return {'x': _w((lambda *s: _rng.normal(s) * 0.05)(B, S, Dm)), 'mem0': _w((lambda *s: _rng.normal(s) * 0.4)(B, M, Dm)), 'Wq': _w((lambda *s: _rng.normal(s) * 3.2)(Dm, H, Dh) * Dm ** (-0.5)), 'Wk': _w((lambda *s: _rng.normal(s) * 3.2)(Dm, H, Dh) * Dm ** (-0.5)), 'Wv': _w((lambda *s: _rng.normal(s) * 0.4)(Dm, H, Dh) * Dm ** (-0.5)), 'Wo': _w((lambda *s: _rng.normal(s) * 0.4)(H, Dh, Dm) * (H * Dh) ** (-0.5)), 'seg_len': seg}
    _B_in = _B_setup()
    return {'A_q': _A_in['q'], 'A_k': _A_in['k'], 'A_v': _A_in['v'], 'A_shift_k': _A_in['shift_k'], 'A_ssm_k': _A_in['ssm_k'], 'A_ssm_D': _A_in['ssm_D'], 'B_x': _B_in['x'], 'B_mem0': _B_in['mem0'], 'B_Wq': _B_in['Wq'], 'B_Wk': _B_in['Wk'], 'B_Wv': _B_in['Wv'], 'B_Wo': _B_in['Wo'], 'B_seg_len': _B_in['seg_len'], 'gate_w': _w((lambda *s: _rng.normal(s) * 0.05)(1024) * 16.0)}

def reference(A_q, A_k, A_v, A_shift_k, A_ssm_k, A_ssm_D, B_x, B_mem0, B_Wq, B_Wk, B_Wv, B_Wo, B_seg_len, gate_w):

    def _A_ref(q, k, v, shift_k, ssm_k, ssm_D):
        B, S, D = q.shape
        ks = shift_k.shape[-1]
        k_pad = jnp.pad(k, ((0, 0), (ks - 1, 0), (0, 0)))
        k_shift = jnp.zeros_like(k)
        for t in range(ks):
            k_shift = k_shift + k_pad[:, t:t + S, :] * shift_k[:, ks - 1 - t][None, None, :]
        kv = k_shift * v
        L = 2 * S
        kv_pad = jnp.pad(kv, ((0, 0), (0, S), (0, 0)))
        kf_pad = jnp.pad(ssm_k, ((0, 0), (0, S)))
        kv_f = (lambda x, axes=(-2, -1): jnp.fft.rfft2(x.astype(jnp.float32), axes=axes))(kv_pad[:, None, :, :], axes=(1, 2))
        kf_f = (lambda x, axes=(-2, -1): jnp.fft.rfft2(x.astype(jnp.float32), axes=axes))(kf_pad[:, None, :], axes=(1, 2))
        kf_f = (lambda x, *d: x.transpose(*d))(kf_f, 1, 2, 0)
        y_f = kv_f * kf_f[None, :, :, :]
        y = (lambda x, s, axes=(-2, -1): jnp.fft.irfft2(x, s=s, axes=axes).astype(jnp.bfloat16))(y_f, (1, L), axes=(1, 2))[:, 0, :S, :]
        y = y + kv * ssm_D[None, None, :]
        return q * y

    def _B_ref(x, mem0, Wq, Wk, Wv, Wo, seg_len):
        B, S, Dm = x.shape
        H, Dh = (Wq.shape[1], Wq.shape[2])
        M = mem0.shape[1]
        scale = Dh ** (-0.5)
        n_seg = S // seg_len
        L = M + seg_len
        idx = jnp.arange(L)
        mask = (idx[:, None] < M) | (idx[:, None] >= idx[None, :])
        mem = mem0
        outs = []
        for s in range(n_seg):
            xs = x[:, s * seg_len:(s + 1) * seg_len, :].copy()
            h = jnp.concatenate([mem, xs], axis=1)
            q = jnp.einsum('btd,dhe->bhte', h, Wq)
            k = jnp.einsum('btd,dhe->bhte', h, Wk)
            v = jnp.einsum('btd,dhe->bhte', h, Wv)
            scores = jnp.einsum('bhqe,bhke->bhqk', q, k) * scale
            scores = jnp.where(mask[None, None], scores, -1000000000.0)
            p = _softmax(scores, axis=-1)
            o = jnp.einsum('bhqk,bhke->bhqe', p, v)
            o = jnp.einsum('bhte,hed->btd', o, Wo)
            mem = o[:, :M, :].copy()
            outs.append(o[:, M:, :])
        return jnp.concatenate(outs, axis=1)
    x = A_q
    g = _sigmoid((x * gate_w).sum(-1, keepdims=True))
    a = _A_ref(x, A_k, A_v, A_shift_k, A_ssm_k, A_ssm_D)
    b = _B_ref(x, B_mem0, B_Wq, B_Wk, B_Wv, B_Wo, B_seg_len)
    return g * a + (1 - g) * b
```

```python
import functools
import math

import jax
import jax.numpy as jnp
import numpy as np
from jax import lax
import jax.experimental.pallas as pl
import jax.experimental.pallas.tpu as pltpu

bf16, f32, u32 = jnp.bfloat16, jnp.float32, jnp.uint32

S, D, H, DH, M, SEG, KS = 2048, 1024, 32, 128, 8, 32, 4
NSEG = S // SEG
L = SEG + M
T = 24
PRE = S - NSEG * T
NC = D // 128
BK = 128
NB = S // BK
NP = BK // 8
HPI = H // NC
ORING = 768
GS = 4


def _dft_matrices():
    ks = np.concatenate([np.arange(0, BK, 2), np.arange(1, BK, 2)])
    n = np.arange(BK)
    ang = np.pi * (2 * ks[:, None] + 1) * n[None, :] / (2 * BK)
    re = np.cos(ang).reshape(NP, 8, BK)
    im = (-np.sin(ang)).reshape(NP, 8, BK)
    fm = np.concatenate([re, im], axis=1).reshape(2 * BK, BK)
    return fm.astype(np.float32), (fm.T / BK).astype(np.float32)


def _kernel(x_hbm, k_hbm, v_hbm, hk_hbm, wq_hbm, wk_hbm, wv_hbm, wo_hbm,
            sk_ref, dd_ref, gw_ref, mem0_ref, f_ref, g_ref,
            out_hbm,
            x_v, w_v, wo_v, qb, kb, vb, ob, mem_v, lo_v, a_v, out_v,
            kc, vc, xc, hc, kf, kvb, ub, hb, zb, skt,
            sem_x, sem_w, sem_wo, sem_c, sem_o):
    W = lambda val: pltpu.bitcast(val, bf16)

    XR = (S - PRE) // NC

    def x_copy0():
        return pltpu.make_async_copy(x_hbm.at[pl.ds(0, PRE), :], x_v.at[pl.ds(0, PRE), :], sem_x.at[NC])

    def x_copy(c):
        rows = pl.ds(pl.multiple_of(PRE + c * XR, 64), XR)
        return pltpu.make_async_copy(x_hbm.at[rows, :], x_v.at[rows, :], sem_x.at[c])

    w_u32 = [w.bitcast(u32) for w in (wq_hbm, wk_hbm, wv_hbm)]

    def w_copies(c):
        cps = []
        for jj in range(HPI // 2):
            j = c * (HPI // 2) + jj
            for m in range(3):
                for par in range(2):
                    cps.append(pltpu.make_async_copy(
                        w_u32[m].at[:, par, j, :], w_v.at[m, 2 * j + par], sem_w.at[c]))
        return cps

    def c_copies(c, slot):
        col = pl.ds(pl.multiple_of(c * 128, 128), 128)
        return [
            pltpu.make_async_copy(hk_hbm.at[col, :], hc.at[slot], sem_c.at[slot, 0]),
            pltpu.make_async_copy(k_hbm.at[:, col], kc.at[slot], sem_c.at[slot, 1]),
            pltpu.make_async_copy(v_hbm.at[:, col], vc.at[slot], sem_c.at[slot, 2]),
            pltpu.make_async_copy(x_hbm.at[:, col], xc.at[slot], sem_c.at[slot, 3]),
        ]

    wo_u32 = wo_hbm.bitcast(u32)

    def wo_copy(n):
        col = pl.ds(pl.multiple_of(n * 128, 128), 128)
        return pltpu.make_async_copy(wo_u32.at[:, col], wo_v.at[n], sem_wo.at[n])

    for cp in c_copies(0, 0):
        cp.start()
    x_copy0().start()
    for cp in w_copies(0):
        cp.start()

    eye = (lax.broadcasted_iota(jnp.int32, (8, KS), 0)
           == lax.broadcasted_iota(jnp.int32, (8, KS), 1)).astype(bf16)
    skt_val = lax.dot_general(eye, sk_ref[...], (((1,), (1,)), ((), ())), preferred_element_type=f32)
    dd_val = dd_ref[...].astype(f32)
    for c in range(NC):
        skt[c, 0:8, :] = skt_val[:, c * 128:(c + 1) * 128]
        skt[c, 8:16, :] = jnp.broadcast_to(dd_val[:, c * 128:(c + 1) * 128], (8, 128))
    kf[0:8, :] = jnp.zeros((8, 128), f32)
    mem_v[...] = mem0_ref[...]

    x_copy0().wait()

    def prologue(c, carry):
        slot = lax.rem(c, 2)
        for cp in c_copies(c, slot):
            cp.wait()
        for cp in w_copies(c):
            cp.wait()

        @pl.when(c + 1 < NC)
        def _():
            for cp in c_copies(c + 1, 1 - slot):
                cp.start()
            for cp in w_copies(c + 1):
                cp.start()

        x_copy(c).start()
        wo_copy(c).start()

        fm = f_ref[...]
        gm = g_ref[...]

        def relayout(m, jj):
            j = c * (HPI // 2) + jj
            a = w_v[m, 2 * j]
            b = w_v[m, 2 * j + 1]
            w_v[m, 2 * j] = (a & u32(0xFFFF)) | (b << 16)
            w_v[m, 2 * j + 1] = (a >> 16) | (b & u32(0xFFFF0000))

        def proj(m, hh):
            h = c * HPI + hh
            dst = (qb, kb, vb)[m]
            r = jnp.dot(x_v[0:PRE, :], W(w_v[m, h]), preferred_element_type=f32)
            dst[h, 0:PRE, :] = r.astype(bf16)

        def conv_h():
            for m in range(NB):
                hb[m] = lax.dot_general(fm, hc[slot, :, m * BK:(m + 1) * BK],
                                        (((1,), (1,)), ((), ())), preferred_element_type=f32)

        def conv_u():
            sk = [skt[c, j:j + 1, :] for j in range(KS)]
            for i in range(NB):
                kf[8 + i * BK:8 + (i + 1) * BK, :] = kc[slot, i * BK:(i + 1) * BK, :].astype(f32)
            for i in range(NB):
                ks = kf[8 + i * BK:8 + (i + 1) * BK, :] * sk[0]
                for j in range(1, KS):
                    ks = ks + kf[8 - j + i * BK:8 - j + (i + 1) * BK, :] * sk[j]
                kv = (ks * vc[slot, i * BK:(i + 1) * BK, :].astype(f32)).astype(bf16)
                kvb[i * BK:(i + 1) * BK, :] = kv
                ub[i] = jnp.dot(fm, kv, preferred_element_type=f32)

        def conv_mac(p):
            re = slice(p * 16, p * 16 + 8)
            im = slice(p * 16 + 8, p * 16 + 16)
            for m in range(NB - 1, 0, -1):
                hr, hi = hb[m, re, :], hb[m, im, :]
                pr, pi = hb[m - 1, re, :], hb[m - 1, im, :]
                if p < NP // 2:
                    hb[m, re, :] = hr - pi
                    hb[m, im, :] = hi + pr
                else:
                    hb[m, re, :] = hr + pi
                    hb[m, im, :] = hi - pr
            IB = 4
            for i0 in range(0, NB, IB):
                zr = [None] * IB
                zi = [None] * IB
                hw = {}
                for j in range(i0 + IB):
                    ur, ui = ub[j, re, :], ub[j, im, :]
                    for ii in range(IB):
                        m = i0 + ii - j
                        if m < 0:
                            continue
                        if m not in hw:
                            hw[m] = (hb[m, re, :], hb[m, im, :])
                        hr, hi = hw[m]
                        tr = hr * ur - hi * ui
                        ti = hr * ui + hi * ur
                        zr[ii] = tr if zr[ii] is None else zr[ii] + tr
                        zi[ii] = ti if zi[ii] is None else zi[ii] + ti
                for ii in range(IB):
                    z = jnp.concatenate([zr[ii], zi[ii]], axis=0).astype(bf16)
                    zb[i0 + ii, p * 8:(p + 1) * 8, :] = pltpu.bitcast(z, u32)

        def conv_inv():
            dvec = skt[c, 8:9, :]
            for i in range(NB):
                rows = slice(i * BK, (i + 1) * BK)
                y = jnp.dot(gm, W(zb[i]), preferred_element_type=f32)
                y = y + kvb[rows, :].astype(f32) * dvec
                a_v[c, rows, :] = (xc[slot, rows, :].astype(f32) * y).astype(bf16)

        order = [(m, hh) for hh in range(HPI) for m in range(3)]
        order.sort(key=lambda t: (t[1] // 2, t[0], t[1]))
        conv_h()
        laid = set()
        pos = 0
        for n, (m, hh) in enumerate(order):
            if (m, hh // 2) not in laid:
                relayout(m, hh // 2)
                laid.add((m, hh // 2))
            proj(m, hh)
            if n == 0:
                conv_u()
            elif 1 <= n <= 8:
                conv_mac(pos)
                conv_mac(pos + 1)
                pos += 2
            elif n == 9:
                conv_inv()
        return carry

    lax.fori_loop(0, NC, prologue, 0)

    for n in range(NC):
        x_copy(n).wait()
        wo_copy(n).wait()

    scale = DH ** -0.5
    cexp = scale * math.log2(math.e)
    neg = -1000000000.0 / scale
    row = lax.broadcasted_iota(jnp.int32, (L, L), 0)
    col = lax.broadcasted_iota(jnp.int32, (L, L), 1)
    allowed = (col <= row) | (col >= SEG) | (row >= SEG)
    G = H // GS

    def gate_rows(r0, n):
        xr = x_v[pl.ds(r0, n), :].astype(f32) * gw_ref[...].astype(f32)
        return jax.nn.sigmoid(jnp.sum(xr, axis=-1, keepdims=True))

    def combine(r0, n, nt, b, g):
        a = a_v[nt, pl.ds(r0, n), :].astype(f32)
        out_v[pl.ds(r0, n), nt * 128:(nt + 1) * 128] = (b + g * (a - b)).astype(bf16)

    def out_copy(r0, n):
        return pltpu.make_async_copy(out_v.at[pl.ds(r0, n), :], out_hbm.at[pl.ds(r0, n), :], sem_o.at[0])

    def step(s, carry):
        t0 = pl.multiple_of(PRE + T * s, 8)
        a0 = pl.multiple_of(SEG * s, SEG)
        o0 = pl.multiple_of(T * s, 8)
        ow = pl.multiple_of(lax.rem(SEG * s, ORING), SEG)
        orr = pl.multiple_of(lax.rem(T * s, ORING), 8)
        lhs = jnp.concatenate([mem_v[...], x_v[pl.ds(t0, T), :]], axis=0)
        st, pend = {}, {}

        def stage_a(g):
            for h in range(g * GS, (g + 1) * GS):
                r = [jnp.dot(lhs, W(w_v[m, h]), preferred_element_type=f32).astype(bf16) for m in range(3)]
                pend[h] = [t[M:] for t in r]
                st[h] = [t[:M] for t in r]

        def stage_a_store(g):
            for h in range(g * GS, (g + 1) * GS):
                for dst, val in zip((qb, kb, vb), pend.pop(h)):
                    dst[h, pl.ds(t0, T), :] = val

        def stage_b(g):
            scs = []
            for h in range(g * GS, (g + 1) * GS):
                q = jnp.concatenate([qb[h, pl.ds(a0, SEG), :], st[h][0]], axis=0)
                k = jnp.concatenate([kb[h, pl.ds(a0, SEG), :], st[h][1]], axis=0)
                scs.append(lax.dot_general(q, k, (((1,), (1,)), ((), ())), preferred_element_type=f32))
            for h, sc in zip(range(g * GS, (g + 1) * GS), scs):
                sc = jnp.where(allowed, sc, neg)
                mx = jnp.max(sc, axis=-1, keepdims=True)
                p = jnp.exp2((sc - mx) * cexp)
                den = jnp.sum(p, axis=-1, keepdims=True)
                st[h] = [(p * (1.0 / den)).astype(bf16), st[h][2]]

        def stage_c(g):
            outs = []
            for h in range(g * GS, (g + 1) * GS):
                p, vm = st.pop(h)
                v = jnp.concatenate([vb[h, pl.ds(a0, SEG), :], vm], axis=0)
                outs.append(jnp.dot(p, v, preferred_element_type=f32).astype(bf16))
            for h, o in zip(range(g * GS, (g + 1) * GS), outs):
                ob[h, pl.ds(ow, SEG), :] = o[:SEG]
            for h, o in zip(range(g * GS, (g + 1) * GS), outs):
                val = jnp.concatenate([o[SEG:], ob[h, pl.ds(orr, T), :]], axis=0)
                lo_v[h] = pltpu.bitcast(val, u32)

        rs = [None] * NC

        def stage_o(h0, h1):
            lo = jnp.concatenate([W(lo_v[h]) for h in range(h0, h1)], axis=1)
            for n in range(NC):
                r = jnp.dot(lo, W(wo_v[n, h0 * 64:h1 * 64, :]), preferred_element_type=f32)
                rs[n] = r if rs[n] is None else r + rs[n]

        g_rows = gate_rows(o0, T)
        for i in range(G):
            stage_a(i)
            if i >= 1:
                stage_b(i - 1)
            if i >= 2:
                stage_c(i - 2)
            stage_a_store(i)
        stage_o(0, 8)
        stage_b(G - 1)
        stage_c(G - 2)
        stage_o(8, 16)
        stage_c(G - 1)
        stage_o(16, 24)
        stage_o(24, 32)
        for n in range(NC):
            mem_v[:, n * 128:(n + 1) * 128] = rs[n][:M].astype(bf16)
            combine(o0, T, n, rs[n][M:], g_rows)
        out_copy(o0, T).start()
        return carry

    lax.fori_loop(0, NSEG, step, 0)

    FB = 128

    def final(i, carry):
        r0 = pl.multiple_of(NSEG * T + i * FB, FB)
        rr = pl.multiple_of(lax.rem(r0, ORING), FB)
        g_rows = gate_rows(r0, FB)
        lo = jnp.concatenate([ob[h, pl.ds(rr, FB), :] for h in range(H)], axis=1)
        for n in range(NC):
            r = jnp.dot(lo, W(wo_v[n]), preferred_element_type=f32)
            combine(r0, FB, n, r, g_rows)
        out_copy(r0, FB).start()
        return carry

    lax.fori_loop(0, PRE // FB, final, 0)
    out_copy(0, S).wait()


@functools.partial(jax.jit, static_argnames=("B_seg_len",))
def pallas_gated_mix__ssm_conv_h3__memory_aug_recurrent_mem_tr__prompt_kernel(
    A_q: jax.Array,
    A_k: jax.Array,
    A_v: jax.Array,
    A_shift_k: jax.Array,
    A_ssm_k: jax.Array,
    A_ssm_D: jax.Array,
    B_x: jax.Array,
    B_mem0: jax.Array,
    B_Wq: jax.Array,
    B_Wk: jax.Array,
    B_Wv: jax.Array,
    B_Wo: jax.Array,
    B_seg_len,
    gate_w: jax.Array,
):
    del B_x
    assert int(B_seg_len) == SEG
    assert A_q.shape == (1, S, D) and B_Wq.shape == (D, H, DH) and B_mem0.shape == (1, M, D)
    fm, gm = _dft_matrices()
    any_spec = pl.BlockSpec(memory_space=pl.ANY)
    vmem_spec = pl.BlockSpec(memory_space=pltpu.VMEM)
    out = pl.pallas_call(
        _kernel,
        out_shape=jax.ShapeDtypeStruct((S, D), bf16),
        in_specs=[any_spec] * 8 + [vmem_spec] * 6,
        out_specs=any_spec,
        scratch_shapes=[
            pltpu.VMEM((S, D), bf16),
            pltpu.VMEM((3, H, D // 2, DH), u32),
            pltpu.VMEM((NC, H * DH // 2, 128), u32),
            pltpu.VMEM((H, S, DH), bf16),
            pltpu.VMEM((H, S, DH), bf16),
            pltpu.VMEM((H, S, DH), bf16),
            pltpu.VMEM((H, ORING, DH), bf16),
            pltpu.VMEM((M, D), bf16),
            pltpu.VMEM((H, 16, DH), u32),
            pltpu.VMEM((NC, S, 128), bf16),
            pltpu.VMEM((S, D), bf16),
            pltpu.VMEM((2, S, 128), bf16),
            pltpu.VMEM((2, S, 128), bf16),
            pltpu.VMEM((2, S, 128), bf16),
            pltpu.VMEM((2, 128, S), bf16),
            pltpu.VMEM((S + 8, 128), f32),
            pltpu.VMEM((S, 128), bf16),
            pltpu.VMEM((NB, 2 * BK, 128), f32),
            pltpu.VMEM((NB, 2 * BK, 128), f32),
            pltpu.VMEM((NB, BK, 128), u32),
            pltpu.VMEM((NC, 16, 128), f32),
            pltpu.SemaphoreType.DMA((NC + 1,)),
            pltpu.SemaphoreType.DMA((NC,)),
            pltpu.SemaphoreType.DMA((NC,)),
            pltpu.SemaphoreType.DMA((2, 4)),
            pltpu.SemaphoreType.DMA((1,)),
        ],
        compiler_params=pltpu.CompilerParams(vmem_limit_bytes=124 * 2**20),
    )(
        A_q.reshape(S, D), A_k.reshape(S, D), A_v.reshape(S, D), A_ssm_k,
        B_Wq.reshape(D // 2, 2, H, DH), B_Wk.reshape(D // 2, 2, H, DH), B_Wv.reshape(D // 2, 2, H, DH),
        B_Wo.reshape(H * DH, D),
        A_shift_k, A_ssm_D.reshape(1, D), gate_w.reshape(1, D), B_mem0.reshape(M, D),
        jnp.asarray(fm, bf16), jnp.asarray(gm, bf16),
    )
    return out.reshape(1, S, D)
```

```python
import math

import jax
import jax.numpy as jnp
import numpy as np
from jax import lax
import jax.experimental.pallas as pl
import jax.experimental.pallas.tpu as pltpu

bf16, f32, u32 = jnp.bfloat16, jnp.float32, jnp.uint32

S, D, H, DH, M, SEG, KS = 2048, 1024, 32, 128, 8, 32, 4
NSEG = S // SEG
L = SEG + M
T = 24
NPAIR = NSEG // 2
PRE = S - NSEG * T
NC = D // 128
BK = 128
NB = S // BK
NP = BK // 8
HPI = H // NC
GS = 4
LAGB, LAGC = 1, 2
EARLY_O = {6: 4}
TAIL = (6, 10, 8, 4)
PART1 = [(0, 0), (1, 0), (2, 0)]
PART2 = [(0, 1), (1, 1), (2, 1)]
UNROLL = 2
SLOW = 4
INV_AFTER = {0: range(0, 5), 1: range(5, 6), 2: range(6, 10), 3: range(10, 11), 4: range(11, 12),
             5: range(12, 13), 6: range(13, 16)}
KSPLIT = 2


def _dft_matrices():
    ks = np.concatenate([np.arange(0, BK, 2), np.arange(1, BK, 2)])
    om = np.pi * (2 * ks[:, None] + 1) / (2 * BK)
    fms = []
    for shift in (0.0, (BK - 1) / 2):
        ang = om * (np.arange(BK)[None, :] - shift)
        re = np.cos(ang).reshape(NP, 8, BK)
        im = (-np.sin(ang)).reshape(NP, 8, BK)
        fms.append(np.concatenate([re, im], axis=1).reshape(2 * BK, BK))
    ang = (om * (np.arange(BK // 2)[None, :] - (BK - 1) / 2)).T
    gm = np.stack([np.cos(ang), np.sin(ang)]) / BK
    return np.stack(fms).astype(np.float32), gm.astype(np.float32)


def _kernel(x_hbm, k_hbm, v_hbm, hk_hbm, wq_hbm, wk_hbm, wv_hbm, wo_hbm,
            sk_hbm, dd_hbm, gw_hbm, mem0_hbm, f_hbm, g_hbm,
            out_hbm,
            xt, xb, w_v, wo_v, qb, kb, vb, ob, mem_v, a_v, out_t, out_b, sq, so,
            kc, vc, hc, kf, kvb, ub, hp, zb, skt,
            sk_ref, dd_ref, gw_ref, m0_ref, f_ref, g_ref,
            sem_x, sem_w, sem_wo, sem_c, sem_o, sem_s, sem_f):
    W = lambda val: pltpu.bitcast(val, bf16)
    F = lambda val: pltpu.bitcast(val, bf16).astype(f32)
    U = lambda ref: ref.bitcast(u32)

    def stage(ref, idx, val):
        ref[idx] = val.astype(bf16)
        return U(ref)[idx]

    cat0 = lambda *vals: jnp.concatenate(vals, axis=0)

    halves = ((0, 0), (M, 2 * SEG - M))

    def xb_copies():
        return [pltpu.make_async_copy(x_hbm.at[:, pl.ds(src, M), pl.ds(n * 128, 128)],
                                      xb.at[n, :, pl.ds(dst, M), :], sem_x.at[NC])
                for n in range(NC) for dst, src in halves]

    def x_copy(c):
        col = pl.ds(pl.multiple_of(c * 128, 128), 128)
        return pltpu.make_async_copy(x_hbm.at[:, :, col], xt.at[c], sem_x.at[c])

    w_u32 = [w.bitcast(u32) for w in (wq_hbm, wk_hbm, wv_hbm)]

    def w_copies(c, which, sem_of=lambda m, jj: int((m, jj) in PART2)):
        cps = []
        for jj in range(HPI // 2):
            j = c * (HPI // 2) + jj
            for m in range(3):
                if (m, jj) not in which:
                    continue
                for par in range(2):
                    cps.append(pltpu.make_async_copy(
                        w_u32[m].at[:, par, j, :], w_v.at[m, 2 * j + par], sem_w.at[c, sem_of(m, jj)]))
        return cps

    def c_copies(c, first=0):
        col = pl.ds(pl.multiple_of(c * 128, 128), 128)
        return [
            pltpu.make_async_copy(hk_hbm.at[col, :], hc, sem_c.at[first]),
            pltpu.make_async_copy(k_hbm.at[:, col], kc, sem_c.at[0]),
            pltpu.make_async_copy(v_hbm.at[:, col], vc, sem_c.at[0]),
        ]

    small = [pltpu.make_async_copy(src, dst, sem_s.at[i]) for i, (src, dst) in enumerate(
        [(f_hbm, f_ref), (sk_hbm, sk_ref), (dd_hbm, dd_ref), (g_hbm, g_ref), (gw_hbm, gw_ref), (mem0_hbm, m0_ref)])]

    def wo_copy(n):
        col = pl.ds(pl.multiple_of(n * 128, 128), 128)
        return pltpu.make_async_copy(wo_hbm.at[:, col], wo_v.at[n], sem_wo.at[n])

    def start_all(cps, priority=0):
        for cp in cps:
            cp.start(priority=priority)

    def wait_all(cps):
        for cp in cps:
            cp.wait()

    def prologue_ops(c):
        link = [None]
        zero = pltpu.bitcast(kf[0:8, :], u32)

        def relayout(m, jj):
            j = c * (HPI // 2) + jj
            a = w_v[m, 2 * j]
            b = w_v[m, 2 * j + 1]
            w_v[m, 2 * j] = (a & u32(0xFFFF)) | (b << 16)
            w_v[m, 2 * j + 1] = (a >> 16) | (b & u32(0xFFFF0000))

        def proj(m, hh):
            h = c * HPI + hh
            dst = (qb, kb, vb)[m]
            x0 = jnp.concatenate([W(U(xb)[n].reshape(PRE // 2, 128)) for n in range(NC)], axis=1)
            r = jnp.dot(x0, W(w_v[m, h]), preferred_element_type=f32)
            dst[h] = r.astype(bf16)

        def conv_h():
            fm = f_ref[0]
            prev = None
            for m in range(NB):
                cur = lax.dot_general(fm, hc[:, m * BK:(m + 1) * BK],
                                      (((1,), (1,)), ((), ())), preferred_element_type=f32)
                if prev is None:
                    hp[m] = cur
                else:
                    for p in range(NP):
                        re = slice(p * 16, p * 16 + 8)
                        im = slice(p * 16 + 8, p * 16 + 16)
                        hp[m, re, :] = cur[re] - prev[im] if p < NP // 2 else cur[re] + prev[im]
                        hp[m, im, :] = cur[im] + prev[re] if p < NP // 2 else cur[im] - prev[re]
                prev = cur

        def conv_u():
            fm = f_ref[1]
            sk = [skt[c, j:j + 1, :] for j in range(KS)]
            for i in range(NB):
                kf[8 + i * BK:8 + (i + 1) * BK, :] = F(U(kc)[i * BK // 2:(i + 1) * BK // 2, :])
            for i in range(NB):
                ks = kf[8 + i * BK:8 + (i + 1) * BK, :] * sk[0]
                for j in range(1, KS):
                    ks = ks + kf[8 - j + i * BK:8 - j + (i + 1) * BK, :] * sk[j]
                kv = stage(kvb, i, ks * F(U(vc)[i * BK // 2:(i + 1) * BK // 2, :]))
                ub[i] = jnp.dot(fm, W(kv), preferred_element_type=f32)

        def conv_mac(i):
            for p in range(NP):
                re = slice(p * 16, p * 16 + 8)
                im = slice(p * 16 + 8, p * 16 + 16)
                zr = zi = None
                for j in range(i, -1, -1):
                    m = i - j
                    ur, ui = ub[j, re, :], ub[j, im, :]
                    hr, hi = hp[m, re, :], hp[m, im, :]
                    if zr is None:
                        zr, zi = hr * ur, hr * ui
                        if link[0] is not None:
                            zr = pltpu.bitcast(pltpu.bitcast(zr, u32) | link[0], f32)
                            zi = pltpu.bitcast(pltpu.bitcast(zi, u32) | link[0], f32)
                        zr = zr - hi * ui
                        zi = zi + hi * ur
                    elif m % SLOW == 0:
                        zr = (zr + hr * ur) - hi * ui
                        zi = (zi + hr * ui) + hi * ur
                    else:
                        zr = zr + (hr * ur - hi * ui)
                        zi = zi + (hr * ui + hi * ur)
                link[0] = (pltpu.bitcast(zr, u32) | pltpu.bitcast(zi, u32)) & zero
                if p % 2 == 0:
                    prev = (zr, zi)
                else:
                    for t, (za, zc) in enumerate(zip(prev, (zr, zi))):
                        zb[i, t, (p - 1) * 8:(p + 1) * 8, :] = cat0(za, zc).astype(bf16)

        def conv_inv(blocks):
            ge, go = g_ref[0], g_ref[1]
            dvec = skt[c, KS:KS + 1, :]
            rev = 7 - lax.broadcasted_iota(jnp.int32, (8, 128), 0)
            hb2 = BK // 2
            for i in blocks:
                ev = jnp.dot(ge, W(U(zb)[i, 0]), preferred_element_type=f32)
                od = jnp.dot(go, W(U(zb)[i, 1]), preferred_element_type=f32)
                hi_rev = ev + od
                hi = jnp.concatenate(
                    [jnp.take_along_axis(hi_rev[hb2 - 8 * (v + 1):hb2 - 8 * v], rev, axis=0)
                     for v in range(hb2 // 8)], axis=0)
                y = jnp.concatenate([ev - od, hi], axis=0)
                a_v[c, i * BK:(i + 1) * BK, :] = (y + F(U(kvb)[i]) * dvec).astype(bf16)

        return relayout, proj, conv_h, conv_u, conv_mac, conv_inv

    def fence():
        pl.semaphore_signal(sem_f, 1)
        pl.semaphore_wait(sem_f, 1)

    cc0 = c_copies(0, first=1)
    wq0 = w_copies(0, [(0, 0)], lambda m, jj: 2)
    wk0 = w_copies(0, [(1, 0)])
    wv0 = w_copies(0, [(2, 0)], lambda m, jj: 3)
    start_all(xb_copies() + wq0)
    fence()
    start_all(small + cc0[:1] + wk0)
    fence()
    start_all(cc0[1:] + wv0)
    fence()
    start_all(w_copies(0, PART2))
    kf[0:8, :] = jnp.zeros((8, 128), f32)
    wait_all(xb_copies() + wq0)
    relayout, proj, conv_h, conv_u, conv_mac, conv_inv = prologue_ops(0)
    relayout(0, 0)
    proj(0, 0)
    proj(0, 1)
    wait_all(small + cc0[:1] + wk0)
    skt_val = sk_ref[...].astype(f32)
    dd_val = dd_ref[...].astype(f32)
    for c in range(NC):
        skt[c, 0:KS, :] = skt_val[:, c * 128:(c + 1) * 128]
        skt[c, KS:KS + 1, :] = dd_val[c:c + 1, :]
        m0 = m0_ref[:, c * 128:(c + 1) * 128].astype(f32)
        mem_v[0, c] = cat0(m0, m0).astype(bf16)
    conv_h()
    relayout(1, 0)
    proj(1, 0)
    proj(1, 1)
    start_all(w_copies(1, PART1))
    start_all([x_copy(0), wo_copy(0)], priority=1)
    wait_all(cc0[1:] + wv0)
    relayout(2, 0)
    proj(2, 0)
    conv_u()
    start_all(c_copies(1))

    def prologue(c, carry):
        wait_all(w_copies(c, PART2))
        relayout, proj, _, _, conv_mac, conv_inv = prologue_ops(c)
        for i in range(NB):
            conv_mac(i)
        for n, (m, hh) in enumerate([(2, 1), (0, 2), (0, 3), (1, 2), (1, 3), (2, 2), (2, 3)]):
            if hh % 2 == 0:
                relayout(m, hh // 2)
            proj(m, hh)
            conv_inv(INV_AFTER.get(n, ()))

        @pl.when(c != NC - 1)
        def _():
            start_all(w_copies(c + 1, PART2))
            start_all([x_copy(c + 1), wo_copy(c + 1)], priority=1)

        @pl.when(c + 1 < NC)
        def _():
            wait_all(w_copies(c + 1, PART1) + c_copies(c + 1))
            relayout, proj, conv_h, conv_u, _, _ = prologue_ops(c + 1)
            relayout(0, 0)
            proj(0, 0)
            conv_h()
            proj(0, 1)
            relayout(1, 0)
            conv_u()
            proj(1, 0)
            proj(1, 1)
            relayout(2, 0)
            proj(2, 0)

            @pl.when(c + 2 < NC)
            def _():
                start_all(w_copies(c + 2, PART1) + c_copies(c + 2))
        return carry

    lax.fori_loop(0, NC, prologue, 0)

    for n in range(NC):
        x_copy(n).wait()
        wo_copy(n).wait()

    scale = DH ** -0.5
    cexp = scale * math.log2(math.e)
    neg = -1000000000.0 / scale
    G = H // GS

    r0_ = lax.broadcasted_iota(jnp.int32, (T + M, L + M), 0)
    c0_ = lax.broadcasted_iota(jnp.int32, (T + M, L + M), 1)
    allowed0 = (c0_ < L) & ((r0_ < M) | (c0_ >= SEG) | (c0_ <= r0_))
    fill0 = jnp.where(c0_ < L, neg, -jnp.inf).astype(f32)
    r1_ = lax.broadcasted_iota(jnp.int32, (L + M, 2 * L), 0)
    c1_ = lax.broadcasted_iota(jnp.int32, (L + M, 2 * L), 1)
    even_r = (r1_ >= SEG) & (r1_ < L)
    even_c = ((c1_ >= SEG) & (c1_ < L)) | (c1_ >= L + M)
    mem_r = (r1_ >= T) & (r1_ < SEG)
    mem_c = ((c1_ >= T) & (c1_ < SEG)) | ((c1_ >= L + M) & (c1_ < L + 2 * M))
    pos = lambda t: jnp.where(t < SEG, t, jnp.where(t < L, t - SEG, jnp.where(t < L + M, t - 2 * M, t - (L + M))))
    in_seg = (even_r & even_c) | (~even_r & ~even_c)
    allowed1 = in_seg & (mem_r | mem_c | (pos(c1_) <= pos(r1_)))
    fill1 = jnp.where(in_seg, neg, -jnp.inf).astype(f32)
    lower = lax.broadcasted_iota(jnp.int32, (8, 128), 0) < 4
    sel = lambda a, b: jnp.where(lower, a, b)

    def gate_of(xs):
        gw = gw_ref[...].astype(f32)
        acc = None
        for nt in range(NC):
            t = F(xs[nt]) * gw[nt:nt + 1, :]
            acc = t if acc is None else acc + t
        return jax.nn.sigmoid(jnp.sum(acc, axis=-1, keepdims=True))

    def combine(x, ya, b, g):
        return (b + g * (F(x) * F(ya) - b)).astype(bf16)

    def softmax(sc, allowed, fill):
        sc = jnp.where(allowed, sc, fill)
        mx = jnp.max(sc, axis=-1, keepdims=True)
        p = jnp.exp2((sc - mx) * cexp)
        den = jnp.sum(p, axis=-1, keepdims=True)
        r = pl.reciprocal(den, approx=True)
        r = r * (2.0 - den * r)
        return (p * r).astype(bf16)

    NT_DIMS = (((1,), (1,)), ((), ()))

    def one_step(par, i, mem, carried, ksplit, ties):
        rows = slice(16 * par, 16 * par + 16)
        bi = pl.ds(pl.multiple_of(8 * i, 8), 8)
        xs = [U(xt)[n, i, rows, :] for n in range(NC)]
        zero = pltpu.bitcast(kf[0:8, :], u32)
        if par == 0:
            blk = [W(cat0(sel(mem[n], xs[n][0:8]), xs[n][8:16] | zero)) for n in range(NC)]
        else:
            blk = [W(cat0(xs[n][0:8] | zero, sel(xs[n][8:16], mem[n]))) for n in range(NC)]
        lhs_lo = jnp.concatenate(blk[:NC // 2], axis=1)
        lhs_hi = jnp.concatenate(blk[NC // 2:], axis=1)
        lhs = jnp.concatenate([lhs_lo, lhs_hi], axis=1)
        mrows = slice(0, M) if par == 0 else slice(T, T + M)
        st, lo_rows = {}, {}
        half = D // 4

        part = {}

        def stage_a(g):
            if g == 0 and ksplit:
                for h in range(KSPLIT):
                    for m in range(3):
                        part[h, m] = jnp.dot(lhs_lo, W(w_v[m, h, :half]), preferred_element_type=f32)
            for h in range(g * GS, (g + 1) * GS):
                r = []
                for m in range(3):
                    if (h, m) in part:
                        t = jnp.dot(lhs_hi, W(w_v[m, h, half:]), preferred_element_type=f32) + part[h, m]
                    else:
                        t = jnp.dot(lhs, W(w_v[m, h]), preferred_element_type=f32)
                    r.append(stage(sq, (par, m, h), t))
                st[h] = r

        def kv_rows(buf, h, cur, idx):
            if par == 0:
                brow = U(buf)[h, bi] | zero
                carried[h, idx] = (cur, brow)
                return W(cat0(cur, brow))
            prev, brow = carried.pop((h, idx))
            return W(cat0(cur, brow, prev))

        def stage_b(g):
            scs = []
            for h in range(g * GS, (g + 1) * GS):
                q = W(st[h][0]) if par == 0 else W(cat0(st[h][0], U(qb)[h, bi]))
                scs.append(lax.dot_general(q, kv_rows(kb, h, st[h][1], 0), NT_DIMS, preferred_element_type=f32))
            for h, sc in zip(range(g * GS, (g + 1) * GS), scs):
                p = softmax(sc, allowed0, fill0) if par == 0 else softmax(sc, allowed1, fill1)
                st[h] = [p, st[h][2]]

        def stage_c(g):
            for h in range(g * GS, (g + 1) * GS):
                p, vm = st.pop(h)
                if h in ties:
                    vm = vm | ties.pop(h)
                o = jnp.dot(p, kv_rows(vb, h, vm, 1), preferred_element_type=f32)
                lo_rows[h] = stage(so, (par, h), o[0:32])
                if par == 1:
                    ob[h, pl.ds(pl.multiple_of(16 * i, 16), 16), :] = o[32:48].astype(bf16)

        rs = [None] * NC

        def stage_o(h0, h1):
            lo = jnp.concatenate([W(lo_rows.pop(h)) for h in range(h0, h1)], axis=1)
            for n in range(NC):
                r = jnp.dot(lo, W(U(wo_v)[n, h0 * 64:h1 * 64, :]), preferred_element_type=f32)
                rs[n] = r if rs[n] is None else r + rs[n]

        g_rows = gate_of(xs)
        h0 = 0
        for g in range(G):
            stage_a(g)
            if g >= LAGC:
                stage_c(g - LAGC)
            if g >= LAGB:
                stage_b(g - LAGB)
            if g in EARLY_O:
                stage_o(h0, h0 + EARLY_O[g])
                h0 += EARLY_O[g]
        for t in range(LAGC):
            g = G + t
            stage_o(h0, h0 + TAIL[t])
            h0 += TAIL[t]
            stage_c(g - LAGC)
            if g - LAGB < G:
                stage_b(g - LAGB)
        for tt in TAIL[LAGC:]:
            stage_o(h0, h0 + tt)
            h0 += tt
        assert h0 == H
        new_mem = [stage(mem_v, (1 - par, n), cat0(rs[n][mrows], rs[n][mrows])) for n in range(NC)]
        for n in range(NC):
            ya = U(a_v)[n, pl.ds(pl.multiple_of(32 * i + 16 * par, 16), 16), :]
            out_t[n, i, 32 * par:32 * par + 32, :] = combine(U(xt)[n, i, rows, :], ya, rs[n], g_rows)
            ties[n] = U(out_t)[n, i, rows, :] & cat0(zero, zero)
        return new_mem

    def step(it, carry):
        mem = [U(mem_v)[0, n] for n in range(NC)]
        ties = {}
        for u in range(UNROLL):
            i = it * UNROLL + u
            carried = {}
            mem = one_step(0, i, mem, carried, u > 0, ties)
            mem = one_step(1, i, mem, carried, True, ties)
            assert not carried
        return carry

    lax.fori_loop(0, NPAIR // UNROLL, step, 0)

    mid = pl.ds(M, 2 * T)
    main_out = [pltpu.make_async_copy(out_t.at[n, :, mid, :], out_hbm.at[:, mid, pl.ds(n * 128, 128)], sem_o.at[0])
                for n in range(NC)]
    start_all(main_out)
    FB = 8

    def final(it, carry):
        prs = pl.ds(it * FB, FB)
        xs = [U(xb)[n, prs].reshape(FB * 8, 128) for n in range(NC)]
        g_rows = gate_of(xs)
        brows = pl.ds(pl.multiple_of(it * FB * 8, FB * 8), FB * 8)
        lo = jnp.concatenate([W(U(ob)[h, brows]) for h in range(H)], axis=1)
        for n in range(NC):
            r = jnp.dot(lo, W(U(wo_v)[n]), preferred_element_type=f32)
            av = U(a_v)[n, pl.ds(pl.multiple_of(it * FB * 32, FB * 32), FB * 32), :].reshape(FB, 32, 128)
            ya = jnp.where(lower[None], av[:, 0:8], av[:, 24:32]).reshape(FB * 8, 128)
            out_b[n, prs] = combine(xs[n], ya, r, g_rows).reshape(FB, 16, 128)
        start_all([pltpu.make_async_copy(out_b.at[n, prs, pl.ds(src, M), :],
                                         out_hbm.at[prs, pl.ds(dst, M), pl.ds(n * 128, 128)], sem_o.at[1])
                   for n in range(NC) for src, dst in halves])
        return carry

    lax.fori_loop(0, NPAIR // FB, final, 0)
    wait_all(main_out)
    pltpu.make_async_copy(out_b, out_b, sem_o.at[1]).wait()


@jax.jit
def pallas_gated_mix__ssm_conv_h3__memory_aug_recurrent_mem_tr__prompt_kernel(
    A_q: jax.Array,
    A_k: jax.Array,
    A_v: jax.Array,
    A_shift_k: jax.Array,
    A_ssm_k: jax.Array,
    A_ssm_D: jax.Array,
    B_x: jax.Array,
    B_mem0: jax.Array,
    B_Wq: jax.Array,
    B_Wk: jax.Array,
    B_Wv: jax.Array,
    B_Wo: jax.Array,
    B_seg_len,
    gate_w: jax.Array,
):
    del B_x
    del B_seg_len
    assert A_q.shape == (1, S, D) and B_Wq.shape == (D, H, DH) and B_mem0.shape == (1, M, D)
    fm, gm = _dft_matrices()
    any_spec = pl.BlockSpec(memory_space=pl.ANY)
    out = pl.pallas_call(
        _kernel,
        out_shape=jax.ShapeDtypeStruct((NPAIR, 2 * SEG, D), bf16),
        in_specs=[any_spec] * 14,
        out_specs=any_spec,
        scratch_shapes=[
            pltpu.VMEM((NC, NPAIR, 64, 128), bf16),
            pltpu.VMEM((NC, NPAIR, 16, 128), bf16),
            pltpu.VMEM((3, H, D // 2, DH), u32),
            pltpu.VMEM((NC, H * DH, 128), bf16),
            pltpu.VMEM((H, PRE, DH), bf16),
            pltpu.VMEM((H, PRE, DH), bf16),
            pltpu.VMEM((H, PRE, DH), bf16),
            pltpu.VMEM((H, PRE, DH), bf16),
            pltpu.VMEM((2, NC, 16, 128), bf16),
            pltpu.VMEM((NC, S, 128), bf16),
            pltpu.VMEM((NC, NPAIR, 64, 128), bf16),
            pltpu.VMEM((NC, NPAIR, 16, 128), bf16),
            pltpu.VMEM((2, 3, H, 32, DH), bf16),
            pltpu.VMEM((2, H, 32, DH), bf16),
            pltpu.VMEM((S, 128), bf16),
            pltpu.VMEM((S, 128), bf16),
            pltpu.VMEM((128, S), bf16),
            pltpu.VMEM((S + 8, 128), f32),
            pltpu.VMEM((NB, BK, 128), bf16),
            pltpu.VMEM((NB, 2 * BK, 128), f32),
            pltpu.VMEM((NB, 2 * BK, 128), f32),
            pltpu.VMEM((NB, 2, BK, 128), bf16),
            pltpu.VMEM((NC, 8, 128), f32),
            pltpu.VMEM((KS, D), bf16),
            pltpu.VMEM((NC, 128), bf16),
            pltpu.VMEM((NC, 128), bf16),
            pltpu.VMEM((M, D), bf16),
            pltpu.VMEM((2, 2 * BK, BK), bf16),
            pltpu.VMEM((2, BK // 2, BK), bf16),
            pltpu.SemaphoreType.DMA((NC + 1,)),
            pltpu.SemaphoreType.DMA((NC, 4)),
            pltpu.SemaphoreType.DMA((NC,)),
            pltpu.SemaphoreType.DMA((2,)),
            pltpu.SemaphoreType.DMA((2,)),
            pltpu.SemaphoreType.DMA((6,)),
            pltpu.SemaphoreType.REGULAR,
        ],
        compiler_params=pltpu.CompilerParams(vmem_limit_bytes=100 * 2**20, disable_bounds_checks=True,
                                             disable_semaphore_checks=True),
    )(
        A_q.reshape(NPAIR, 2 * SEG, D), A_k.reshape(S, D), A_v.reshape(S, D), A_ssm_k,
        B_Wq.reshape(D // 2, 2, H, DH), B_Wk.reshape(D // 2, 2, H, DH), B_Wv.reshape(D // 2, 2, H, DH),
        B_Wo.reshape(H * DH, D),
        A_shift_k.T, A_ssm_D.reshape(NC, 128), gate_w.reshape(NC, 128), B_mem0.reshape(M, D),
        jnp.asarray(fm, bf16), jnp.asarray(gm, bf16),
    )
    return out.reshape(1, S, D)
```
